```python
import jax
import jax.numpy as jnp

def _softmax(x, axis=-1):
    return jax.nn.softmax(x, axis=axis)

def _gelu(x):
    return jax.nn.gelu(x, approximate=True)

def _silu(x):
    return jax.nn.silu(x)

def _sigmoid(x):
    return jax.nn.sigmoid(x)

def _layernorm(x, axis=-1, eps=1e-05):
    m = jnp.mean(x, axis=axis, keepdims=True)
    v = jnp.var(x, axis=axis, keepdims=True)
    return (x - m) / jnp.sqrt(v + eps)

def _scatter_add(tgt, idx, src, axis=0):
    return tgt.at[idx].add(src)

def _segment_sum(src, seg, n):
    return jax.ops.segment_sum(src, seg, n)

class _Rng:

    def __init__(self, key):
        self._k = key

    def _next(self):
        self._k, sub = jax.random.split(self._k)
        return sub

    def normal(self, shape):
        return jax.random.normal(self._next(), shape, dtype=jnp.bfloat16)

    def randint(self, lo, hi, shape):
        return jax.random.randint(self._next(), shape, lo, hi, dtype=jnp.int32)

    def uniform(self, shape, lo=0.0, hi=1.0):
        return jax.random.uniform(self._next(), shape, jnp.bfloat16, lo, hi)

    def permutation(self, n):
        return jax.random.permutation(self._next(), n)
kernel_name = 'adaLN_cond__ssm_conv_h3__dense_activation_gelu__prompt'

def setup_inputs():
    _rng = _Rng(jax.random.key(int.from_bytes(__import__("os").urandom(4), "little")))
    _w = lambda a: (lambda t: t.astype(jnp.bfloat16) if jnp.issubdtype(t.dtype, jnp.floating) else t)(jnp.asarray(a))

    def _A_setup():
        B, S, D = (1, 2048, 640)
        ks = 4
        return {'q': _w((lambda *s: _rng.normal(s) * 0.05)(B, S, D)), 'k': _w((lambda *s: _rng.normal(s) * 0.05)(B, S, D)), 'v': _w((lambda *s: _rng.normal(s) * 0.05)(B, S, D)), 'shift_k': _w((lambda *s: _rng.normal(s) * 0.05)(D, ks) * 0.5), 'ssm_k': _w((lambda *s: _rng.normal(s) * 0.05)(D, S) * (1.0 / S ** 0.5)), 'ssm_D': _w((lambda *s: _rng.normal(s) * 0.05)(D))}
    _A_in = _A_setup()

    def _B_setup():
        B, S, D, F = (1, 2048, 640, 1728)
        return {'x': _w((lambda *s: _rng.normal(s) * 0.05)(B, S, D)), 'w1': _w((lambda *s: _rng.normal(s) * 0.05)(D, F) * D ** (-0.5)), 'b1': _w((lambda *s: _rng.normal(s) * 0.05)(F) * 0.01), 'w2': _w((lambda *s: _rng.normal(s) * 0.05)(F, D) * F ** (-0.5)), 'b2': _w((lambda *s: _rng.normal(s) * 0.05)(D) * 0.01)}
    _B_in = _B_setup()
    return {'A_q': _A_in['q'], 'A_k': _A_in['k'], 'A_v': _A_in['v'], 'A_shift_k': _A_in['shift_k'], 'A_ssm_k': _A_in['ssm_k'], 'A_ssm_D': _A_in['ssm_D'], 'B_x': _B_in['x'], 'B_w1': _B_in['w1'], 'B_b1': _B_in['b1'], 'B_w2': _B_in['w2'], 'B_b2': _B_in['b2'], 'c': _w((lambda *s: _rng.normal(s) * 0.05)(1, 640)), 'w_mod': _w((lambda *s: _rng.normal(s) * 0.05)(640, 6 * 640) * 640 ** (-0.5))}

def reference(A_q, A_k, A_v, A_shift_k, A_ssm_k, A_ssm_D, B_x, B_w1, B_b1, B_w2, B_b2, c, w_mod):

    def _A_ref(q, k, v, shift_k, ssm_k, ssm_D):
        B, S, D = q.shape
        ks = shift_k.shape[-1]
        k_pad = jnp.pad(k, ((0, 0), (ks - 1, 0), (0, 0)))
        k_shift = jnp.zeros_like(k)
        for t in range(ks):
            k_shift = k_shift + k_pad[:, t:t + S, :] * shift_k[:, ks - 1 - t][None, None, :]
        kv = k_shift * v
        L = 2 * S
        kv_pad = jnp.pad(kv, ((0, 0), (0, S), (0, 0)))
        kf_pad = jnp.pad(ssm_k, ((0, 0), (0, S)))
        kv_f = (lambda x, axes=(-2, -1): jnp.fft.rfft2(x.astype(jnp.float32), axes=axes))(kv_pad[:, None, :, :], axes=(1, 2))
        kf_f = (lambda x, axes=(-2, -1): jnp.fft.rfft2(x.astype(jnp.float32), axes=axes))(kf_pad[:, None, :], axes=(1, 2))
        kf_f = (lambda x, *d: x.transpose(*d))(kf_f, 1, 2, 0)
        y_f = kv_f * kf_f[None, :, :, :]
        y = (lambda x, s, axes=(-2, -1): jnp.fft.irfft2(x, s=s, axes=axes).astype(jnp.bfloat16))(y_f, (1, L), axes=(1, 2))[:, 0, :S, :]
        y = y + kv * ssm_D[None, None, :]
        return q * y

    def _B_ref(x, w1, b1, w2, b2):
        h = jnp.einsum('bsd,df->bsf', x, w1) + b1
        h = _gelu(h)
        return jnp.einsum('bsf,fd->bsd', h, w2) + b2
    x = A_q
    mod = (_silu(c) @ w_mod).reshape(c.shape[0], 6, 1, -1)
    sa, ca, ga, sb, cb, gb = (mod[:, 0].copy(), mod[:, 1].copy(), mod[:, 2].copy(), mod[:, 3].copy(), mod[:, 4].copy(), mod[:, 5].copy())
    h = _layernorm(x, axis=-1) * (1 + ca) + sa
    x = x + ga * _A_ref(h, A_k, A_v, A_shift_k, A_ssm_k, A_ssm_D)
    h = _layernorm(x, axis=-1) * (1 + cb) + sb
    x = x + gb * _B_ref(h, B_w1, B_b1, B_w2, B_b2)
    return x
```

```python
import functools
import numpy as np
import jax
import jax.numpy as jnp
from jax import lax
import jax.experimental.pallas as pl
import jax.experimental.pallas.tpu as pltpu

S, D, FF = 2048, 640, 1728
C = 128
NC = S // C
N2 = 2 * C
ND = D // 128
HK = (15,13,14,8)
TM = 256
NP = C // 8


def _dft_mats():
    n = np.arange(C, dtype=np.float64)
    f = np.arange(C, dtype=np.float64)
    ang = 2.0 * np.pi * (f[:, None] + 0.5) * n[None, :] / N2
    re = np.cos(ang).reshape(NP, 8, C)
    im = (-np.sin(ang)).reshape(NP, 8, C)
    fwd = np.concatenate([re, im], axis=1).reshape(N2, C)
    inv = (2.0 / N2) * fwd.T
    return fwd.astype(np.float32), inv.astype(np.float32)


_FWD, _INV = _dft_mats()


def _mo(x, n):
    return x if isinstance(x, int) else pl.multiple_of(x, n)


def _pack(m):
    u = m.astype(jnp.bfloat16).view(np.uint16).astype(np.uint32)
    return u[0::2] | (u[1::2] << 16)


def _kernel(q_hbm, k_hbm, v_hbm, shift_ref, ssmk_hbm, dvec_ref, w1_hbm, b1_ref, w2_hbm,
            b2_ref, c_ref, wmod_hbm, f_ref, g_ref, o_hbm,
            q_v, k_v, v_v, ssmk_v, w1t_v, w1_v, w2_v, wmod_v, x1_s, h2_s, g_s, o_v,
            sems, osem, *bufs):
    f32, bf16, u32 = jnp.float32, jnp.bfloat16, jnp.uint32
    xs, ks, zs, kv_s, ys = bufs[0:2], bufs[2:4], bufs[4:6], bufs[6:6 + ND], bufs[6 + ND:]

    def conv_copies(t):
        cs = pl.ds(t * 128, 128)
        return [
            pltpu.make_async_copy(k_hbm.at[:, cs], k_v.at[t, pl.ds(16, S), :], sems.at[3 * t]),
            pltpu.make_async_copy(v_hbm.at[:, cs], v_v.at[t], sems.at[3 * t + 1]),
            pltpu.make_async_copy(ssmk_hbm.at[cs, :], ssmk_v.at[t], sems.at[3 * t + 2]),
        ]

    rest = [
        pltpu.make_async_copy(wmod_hbm, wmod_v, sems.at[3 * ND]),
        pltpu.make_async_copy(q_hbm, q_v, sems.at[3 * ND + 1]),
        pltpu.make_async_copy(w1_hbm, w1t_v, sems.at[3 * ND + 2]),
        pltpu.make_async_copy(w2_hbm, w2_v, sems.at[3 * ND + 3]),
    ]
    for cp in conv_copies(0):
        cp.start()

    for t in range(ND):
        k_v[t, 0:16, :] = jnp.zeros((16, 128), bf16)
    shift_t = shift_ref[...].astype(f32)
    dvec = dvec_ref[...].astype(f32).reshape(1, D)
    flag = lax.broadcasted_iota(jnp.int32,(8,128),0) + (c_ref[...].reshape(1,D)[:, :128] > 0).astype(jnp.int32)
    sgn = (1 - 2 * (lax.broadcasted_iota(jnp.int32, (8, 128), 0) & 1)).astype(f32)

    def kv_stage(t, p):
        cs = slice(t * 128, (t + 1) * 128)
        r = _mo(p * C, C)
        kf = k_v[t, pl.ds(r, C + 16), :].astype(f32)
        acc = kf[16:] * shift_t[0:1, cs]
        for s in range(1, 4):
            acc = acc + kf[16 - s:16 - s + C] * shift_t[s:s + 1, cs]
        kv = (acc * v_v[t, pl.ds(r, C), :].astype(f32)).astype(bf16)
        kv_s[t][pl.ds(_mo(p * (C // 2), C // 2), C // 2), :] = pltpu.bitcast(kv, u32)
        return acc[-8:]

    def load_kv(t, p):
        return pltpu.bitcast(kv_s[t][pl.ds(_mo(p * (C // 2), C // 2), C // 2), :], bf16)

    def fwd_stage(t, p):
        fmat = pltpu.bitcast(f_ref[...], bf16)
        xs[t % 2][p] = r = jnp.dot(fmat, load_kv(t, p), preferred_element_type=f32)
        return r[-8:]

    def fwk_stage(t, p):
        fmat = pltpu.bitcast(f_ref[...], bf16)
        kc = ssmk_v[t, :, pl.ds(_mo(p * C, C), C)]
        ks[t % 2][p] = r = lax.dot_general(fmat, kc, (((1,), (1,)), ((), ())),
                                       preferred_element_type=f32)
        return r[-8:]

    def mac_stage(t, p, hooks):
        b_ = t % 2
        r0 = _mo(p * 16, 16)
        re, im = pl.ds(r0, 8), pl.ds(r0 + 8, 8)
        ka, kb, kab, xc, xdm, xdp = [], [], [], [], [], []
        pr = pi = None
        for i in range(NC):
            a, b = ks[b_][i, re, :], ks[b_][i, im, :]
            if i == 0:
                a2, b2 = a, b
            else:
                a2, b2 = a - sgn * pi, b + sgn * pr
            pr, pi = a, b
            if i in hooks:
                a2 = (hooks[i](), a2)[1]
            ka.append(a2); kb.append(b2); kab.append(a2 + b2)
            c_, d_ = xs[b_][i, re, :], xs[b_][i, im, :]
            xc.append(c_); xdm.append(d_ - c_); xdp.append(c_ + d_)
            t1 = t2 = t3 = None
            for j in range(i + 1):
                u1, u2, u3 = xc[j] * kab[i - j], xdm[j] * ka[i - j], xdp[j] * kb[i - j]
                if t1 is None:
                    t1, t2, t3 = u1, u2, u3
                else:
                    t1, t2, t3 = t1 + u1, t2 + u2, t3 + u3
            z = jnp.concatenate([t1 - t3, t1 + t2], axis=0).astype(bf16)
            zs[b_][i, pl.ds(_mo(p * 8, 8), 8), :] = pltpu.bitcast(z, u32)

    def inv_stage(t, p):
        cs = slice(t * 128, (t + 1) * 128)
        gmat = pltpu.bitcast(g_ref[...], bf16)
        y = jnp.dot(gmat, pltpu.bitcast(zs[t % 2][p], bf16), preferred_element_type=f32)
        ys[t][p // 2, pl.ds(_mo((p % 2) * C, C), C), :] = r = y + load_kv(t, p).astype(f32) * dvec[:, cs]
        return r[-8:]

    for step in range(ND + 3):
        if step < ND:
            for cp in conv_copies(step):
                cp.wait()
        for cp in {0: conv_copies(1) + conv_copies(2), 1: conv_copies(3), 2: conv_copies(4) + rest[:1],
                   3: rest[1:3], 4: rest[3:]}.get(step, []):
            cp.start()

        def body(p, carry, step=step, mac=False):
            hooks = {}
            for at, stage, t in ((HK[0], inv_stage, step - 3), (HK[1], fwd_stage, step - 1),
                                 (HK[2], fwk_stage, step - 1), (HK[3], kv_stage, step)):
                if 0 <= t < ND:
                    hooks[at] = functools.partial(stage, t, p)
            if mac:
                mac_stage(step - 2, p, hooks)
            else:
                for h in hooks.values():
                    h()
            return carry

        for p_ in range(NC):
            body(p_, 0, mac=0 <= step - 2 < ND)
        if False:
            lax.fori_loop(0, NC, functools.partial(body, mac=True), 0)

    for cp in rest[:3]:
        cp.wait()
    cf = c_ref[...].astype(f32)
    sc = (cf * jax.nn.sigmoid(cf)).astype(bf16)
    mod = jnp.dot(jnp.broadcast_to(sc, (16, D)), wmod_v[...], preferred_element_type=f32)[0:1]
    sa, ca, ga, sb, cb, gb = [mod[:, i * D:(i + 1) * D] for i in range(6)]
    b1 = b1_ref[...].astype(f32).reshape(1, FF)
    b2 = b2_ref[...].astype(f32).reshape(1, D)

    def ln(x):
        m = jnp.mean(x, axis=-1, keepdims=True)
        d = x - m
        var = jnp.mean(d * d, axis=-1, keepdims=True)
        return d * lax.rsqrt(var + 1e-5)

    def out_copy(i, slot):
        return pltpu.make_async_copy(o_v.at[slot], o_hbm.at[pl.ds(i * TM, TM), :], osem.at[slot])

    NB = 256

    RB = 32

    def prep(i, r):
        x = q_v[pl.ds(_mo(i * TM + r, RB), RB), :].astype(f32)
        h = ln(x) * ca1 + sa
        x1 = x + ga * (h * jnp.concatenate([y_[i, r:r + RB] for y_ in ys], axis=1))
        h2 = ln(x1) * cb1 + sb
        x1_s[i % 2, r:r + RB, :] = x1
        h2_s[i % 2, r // 2:(r + RB) // 2, :] = pltpu.bitcast(h2.astype(bf16), u32)
        return h2[-8:, -128:]

    for n0 in range(0, FF, 128):
        n1 = min(FF, n0 + 128)
        w1_v[:, n0:n1] = w1t_v[n0:n1, :].astype(f32).T.astype(bf16)
    ca1, cb1 = 1.0 + ca, 1.0 + cb
    for r in range(0, TM, RB):
        prep(0, r)
    rest[3].wait()

    def tile(i, carry):
        slot = i % 2
        nxt = jnp.minimum(i + 1, S // TM - 1)
        h2 = pltpu.bitcast(h2_s[slot], bf16)
        for ci, n0 in enumerate(range(0, FF, NB)):
            n1 = min(FF, n0 + NB)
            a = jnp.dot(h2, w1_v[:, n0:n1],
                                preferred_element_type=f32) + b1[:, n0:n1]
            u = a * (0.7978845608028654 + 0.035677408136300125 * (a * a))
            ha = 0.5 * a
            g_s[:, n0:n1] = (ha * jnp.tanh(u) + ha).astype(bf16)
        o = jnp.dot(g_s[...], w2_v[...], preferred_element_type=f32) + b2
        rows = []
        for r in range(0, TM, RB):
            o_l = o[r:r + RB, :512]
            o_r = o[r:r + RB, 512:]
            o_r = jnp.concatenate([jnp.where(i >= 0, o_r[:8], prep(nxt, r)), o_r[8:]], axis=0)
            rows.append(jnp.concatenate([o_l, o_r], axis=1))
        o = jnp.concatenate(rows, axis=0)
        res = (x1_s[slot] + gb * o).astype(bf16)

        @pl.when(i >= 2)
        def _():
            out_copy(i - 2, slot).wait()

        o_v[slot] = res
        out_copy(i, slot).start()
        return carry

    nt = S // TM
    lax.fori_loop(0, nt, tile, 0)
    out_copy(nt - 2, nt % 2).wait()
    out_copy(nt - 1, (nt - 1) % 2).wait()


@jax.jit
def pallas_adaLN_cond__ssm_conv_h3__dense_activation_gelu__prompt_kernel(
    A_q, A_k, A_v, A_shift_k, A_ssm_k, A_ssm_D, B_x, B_w1, B_b1, B_w2, B_b2, c, w_mod,
):
    bf16, f32 = jnp.bfloat16, jnp.float32
    hbm = pl.BlockSpec(memory_space=pltpu.HBM)
    vm = pl.BlockSpec(memory_space=pltpu.VMEM)
    out = pl.pallas_call(
        _kernel,
        out_shape=jax.ShapeDtypeStruct((S, D), bf16),
        in_specs=[hbm, hbm, hbm, vm, hbm, vm, hbm, vm, hbm, vm, vm, hbm, vm, vm],
        out_specs=hbm,
        scratch_shapes=[
            pltpu.VMEM((S, D), bf16),
            pltpu.VMEM((ND, S + 16, 128), bf16),
            pltpu.VMEM((ND, S, 128), bf16),
            pltpu.VMEM((ND, 128, S), bf16),
            pltpu.VMEM((FF, D), bf16),
            pltpu.VMEM((D, FF), bf16),
            pltpu.VMEM((FF, D), bf16),
            pltpu.VMEM((D, 6 * D), bf16),
            pltpu.VMEM((2, TM, D), f32),
            pltpu.VMEM((2, TM // 2, D), jnp.uint32),
            pltpu.VMEM((TM, FF), bf16),
            pltpu.VMEM((2, TM, D), bf16),
            pltpu.SemaphoreType.DMA((3 * ND + 4,)),
            pltpu.SemaphoreType.DMA((2,)),
        ] + [pltpu.VMEM((NC, N2, 128), f32)] * 4 + [pltpu.VMEM((NC, C, 128), jnp.uint32)] * 2
          + [pltpu.VMEM((S // 2, 128), jnp.uint32)] * ND + [pltpu.VMEM((8, N2, 128), f32)] * ND,
        compiler_params=pltpu.CompilerParams(vmem_limit_bytes=64 * 1024 * 1024),
    )(A_q.reshape(S, D), A_k.reshape(S, D), A_v.reshape(S, D), A_shift_k.T, A_ssm_k,
      A_ssm_D, B_w1.T, B_b1, B_w2, B_b2, c, w_mod,
      jnp.asarray(_pack(_FWD)), jnp.asarray(_pack(_INV)))
    return out.reshape(1, S, D)
```
